```python
import os as _os
_os.environ.setdefault("JAX_PLATFORMS", "cpu")
import jax
import jax.numpy as jnp

def _softmax(x, axis=-1):
    return jax.nn.softmax(x, axis=axis)
def _gelu(x):
    return jax.nn.gelu(x, approximate=True)
def _silu(x):
    return jax.nn.silu(x)
def _sigmoid(x):
    return jax.nn.sigmoid(x)
def _layernorm(x, axis=-1, eps=1e-5):
    m = jnp.mean(x, axis=axis, keepdims=True)
    v = jnp.var(x, axis=axis, keepdims=True)
    return (x - m) / jnp.sqrt(v + eps)
def _scatter_add(tgt, idx, src, axis=0):
    return tgt.at[idx].add(src)
def _segment_sum(src, seg, n):
    return jax.ops.segment_sum(src, seg, n)
class _Rng:
    def __init__(self, key):
        self._k = key
    def _next(self):
        self._k, sub = jax.random.split(self._k)
        return sub
    def normal(self, shape):
        return jax.random.normal(self._next(), shape, dtype=jnp.bfloat16)
    def randint(self, lo, hi, shape):
        return jax.random.randint(self._next(), shape, lo, hi, dtype=jnp.int32)
    def uniform(self, shape, lo=0.0, hi=1.0):
        return jax.random.uniform(self._next(), shape, jnp.bfloat16, lo, hi)
    def permutation(self, n):
        return jax.random.permutation(self._next(), n)


kernel_name = 'standalone__glu_gated_bilinear__prompt'

def setup_inputs():
    _rng = _Rng(jax.random.key(int.from_bytes(__import__("os").urandom(4), "little")))
    _w = (lambda a: (lambda t: t.astype(jnp.bfloat16) if jnp.issubdtype(t.dtype, jnp.floating) else t)(jnp.asarray(a)))
    B, S, D, F = 1, 2048, 640, 1728
    return {
        "x": _w((lambda *s: _rng.normal(s) * 0.05)(B, S, D)),
        "w_gate": _w((lambda *s: _rng.normal(s) * 0.05)(D, F) * (D ** -0.5)),
        "w_up": _w((lambda *s: _rng.normal(s) * 0.05)(D, F) * (D ** -0.5)),
        "w_down": _w((lambda *s: _rng.normal(s) * 0.05)(F, D) * (F ** -0.5)),
    }

def reference(x, w_gate, w_up, w_down):
    g = jnp.einsum("bsd,df->bsf", x, w_gate)
    u = jnp.einsum("bsd,df->bsf", x, w_up)
    h = g * u
    return jnp.einsum("bsf,fd->bsd", h, w_down)
```

```python
import numpy as np
import jax
import jax.numpy as jnp
from jax import lax
import jax.experimental.pallas as pl
import jax.experimental.pallas.tpu as pltpu

def _add(a, b, s=1):
    o = dict(a)
    for k, c in b.items():
        o[k] = o.get(k, 0) + s * c
    return {k: c for k, c in o.items() if c != 0}
def _scale(a, s): return {k: c * s for k, c in a.items()}

def scheme(p, P, N, edges, sign=None):
    sign = sign or {}
    d = {**P, **N}
    nbr = {c: [] for c in d}
    for a, b in edges:
        nbr[a].append(b); nbr[b].append(a)
    beta, extra = {}, {}
    for c in d:
        basis = [d[c]] + [d[o] for o in nbr[c]]
        ex = []
        for i in range(p):
            if len(basis) == p: break
            e = tuple(int(i == j) for j in range(p))
            if np.linalg.matrix_rank(np.array(basis + [e])) == len(basis) + 1:
                basis.append(e); ex.append(e)
        Dm = np.array(basis, dtype=np.float64)
        assert np.linalg.matrix_rank(Dm) == p, (c, basis)
        inv = np.linalg.inv(Dm.T)
        assert np.allclose(inv, np.round(inv)), "non unimodular"
        inv = np.round(inv).astype(int)
        names = [c] + nbr[c] + ex
        for t, nm in enumerate(names):
            beta[(c, nm)] = {(i, c): int(inv[t, i]) for i in range(p) if inv[t, i]}
        extra[c] = ex
    A = lambda m, vec, s=1: {(m, i): s * c for i, c in enumerate(vec) if c}
    prods = {}
    for a, b in edges:
        s = sign.get((a, b), 1)
        prods[("M1", a, b)] = (_add(A(0, d[a], s), A(1, d[b])), _add(beta[(b, a)], beta[(a, b)]), {(0, b): s, (1, a): 1})
        prods[("M2", a, b)] = (_add(A(1, d[a], s), A(1, d[b])), beta[(b, a)], {(1, b): s, (1, a): -1})
        prods[("M5", a, b)] = (_add(A(0, d[a], s), A(0, d[b])), beta[(a, b)], {(0, b): -s, (0, a): 1})
    for a in P:
        v3, v6 = beta[(a, a)], beta[(a, a)]
        for b in nbr[a]:
            s = sign.get((a, b), 1)
            v3 = _add(v3, beta[(a, b)], -s); v6 = _add(v6, beta[(b, a)], s)
        prods[("M3", a)] = (A(0, d[a]), v3, {(0, a): 1, (1, a): 1})
        prods[("M6", a)] = (_add(A(1, d[a]), A(0, d[a]), -1), v6, {(1, a): 1})
    for b in N:
        v4, v7 = beta[(b, b)], beta[(b, b)]
        for a in nbr[b]:
            s = sign.get((a, b), 1)
            v4 = _add(v4, beta[(b, a)], -s); v7 = _add(v7, beta[(a, b)], s)
        prods[("M4", b)] = (A(1, d[b]), v4, {(0, b): 1, (1, b): 1})
        prods[("M7", b)] = (_add(A(0, d[b]), A(1, d[b]), -1), v7, {(0, b): 1})
    for c in d:
        for e in extra[c]:
            for m in (0, 1):
                prods[("X", c, e, m)] = (A(m, e), beta[(c, e)], {(m, c): 1})
    return prods

def verify(p, cols, prods):
    T = {}
    for u, v, w in prods.values():
        for (m, i), a in u.items():
            for (k, c), b in v.items():
                for (m2, c2), g in w.items():
                    key = (m, i, k, c, m2, c2)
                    T[key] = T.get(key, 0) + a * b * g
    T = {k: x for k, x in T.items() if x}
    want = {(m, i, i, c, m, c): 1 for m in (0, 1) for i in range(p) for c in cols}
    assert T == want, "identity fails"
    return True


E = lambda p, i: tuple(int(i == j) for j in range(p))
def full_group(p, Pc, Nc):
    P = {c: E(p, i) for i, c in enumerate(Pc)}; N = {c: E(p, i) for i, c in enumerate(Nc)}
    edges = [(a, b) for i, a in enumerate(Pc) for j, b in enumerate(Nc) if i != j]
    return scheme(p, P, N, edges)

NT = (((1,), (1,)), ((), ()))
NN = (((1,), (0,)), ((), ()))
f32 = jnp.float32
bf16 = jnp.bfloat16
ANY = pl.BlockSpec(memory_space=pl.ANY)
nt = lambda a, b: lax.dot_general(a, b, NT, preferred_element_type=f32)
nn = lambda a, b: lax.dot_general(a, b, NN, preferred_element_type=f32)
T = 128

def canon(d):
    items = sorted(d.items())
    s = 1 if items[0][1] > 0 else -1
    return tuple((k, c * s) for k, c in items), s

def lincomb(pattern, get):
    pos = [(k, c) for k, c in pattern if c > 0]; neg = [(k, c) for k, c in pattern if c < 0]
    acc = None
    for k, c in pos + neg:
        t = get(k)
        if abs(c) != 1: t = t * float(abs(c))
        if acc is None: acc = t if c > 0 else -t
        elif c > 0: acc = acc + t
        else: acc = acc - t
    return acc

def accum(acc, o, p, c):
    if o not in acc: acc[o] = (p, c); return
    a, s = acc[o]
    if s == c: acc[o] = (a + p, s)
    elif s > 0: acc[o] = (a - p, 1)
    else: acc[o] = (p - a, 1)

def order_s1(prods, P, N, mode):
    keys = list(prods)
    if mode == "byP":
        out = []
        for a in P:
            out += [k for k in keys if k[0] == "M3" and k[1] == a]
            nb = [k[2] for k in keys if k[0] == "M1" and k[1] == a]
            for b in nb: out += [("M5", a, b), ("M1", a, b)]
            out += [k for k in keys if k[0] == "M6" and k[1] == a]
            for b in nb: out += [("M2", a, b)]
            out += [k for k in keys if k[0] == "X" and k[1] == a]
        for b in N:
            out += [("M4", b), ("M7", b)] + [k for k in keys if k[0] == "X" and k[1] == b]
    elif mode == "rawfirst":
        out = []
        for a in P: out += [("M3", a)] + [k for k in keys if k[0] == "M5" and k[1] == a] + [k for k in keys if k[0] == "X" and k[1] == a]
        for b in N: out += [("M4", b)] + [k for k in keys if k[0] == "M2" and k[2] == b] + [k for k in keys if k[0] == "X" and k[1] == b]
        for a in P: out += [("M6", a)] + [k for k in keys if k[0] == "M1" and k[1] == a]
        for b in N: out += [("M7", b)]
    elif mode == "GU":
        out = []
        for a in P: out += [("M3", a)] + [k for k in keys if k[0] == "M5" and k[1] == a] + [k for k in keys if k[0] == "X" and k[1] == a]
        for b in N:
            out += [("M4", b)] + [k for k in keys if k[0] == "M2" and k[2] == b] + [k for k in keys if k[0] == "X" and k[1] == b]
            out += [k for k in keys if k[0] == "M1" and k[2] == b] + [("M7", b)]
        for a in P: out += [("M6", a)]
    elif mode == "GU2":
        out = []
        for a in P: out += [("M3", a)] + [k for k in keys if k[0] == "M5" and k[1] == a] + [k for k in keys if k[0] == "X" and k[1] == a]
        for b in N:
            out += [("M4", b), ("M7", b)] + [k for k in keys if k[0] == "X" and k[1] == b]
            for k in keys:
                if k[0] == "M2" and k[2] == b: out += [k, ("M1",) + k[1:]]
        for a in P: out += [("M6", a)]
    assert sorted(map(str, out)) == sorted(map(str, keys))
    return out

def plan(o1):
    s1 = []
    for f0 in (0, 5):
        Pc = [("g", f0 + i) for i in range(5)]; Nc = [("u", f0 + i) for i in range(5)]
        g = full_group(5, Pc, Nc); verify(5, Pc + Nc, g)
        s1.append((Pc, Nc, g, order_s1(g, Pc, Nc, o1)))
    P = {("g", 10 + i): E(5, i) for i in range(3)}
    N = {("u", 10): E(5, 1), ("u", 11): E(5, 2), ("u", 12): E(5, 3), ("t", 13): E(5, 4)}
    edges = [(a, b) for a in P for b in N if P[a] != N[b]]
    g = scheme(5, P, N, edges); verify(5, list(P) + list(N), g)
    s1.append((list(P), list(N), g, order_s1(g, list(P), list(N), o1)))
    return s1

def plan2():
    P = {0: E(5,0), 1: E(5,1), 2: E(5,2), 3: E(5,3), 4: E(5,4)}
    N = {5: E(5,0), 6: E(5,1), 7: E(5,2), 8: E(5,3), 9: E(5,4)}
    edges = [(a, b) for a in P for b in N if P[a] != N[b]]
    P.update({10: E(5,0), 11: E(5,1)}); N.update({12: E(5,2), 13: E(5,3)})
    edges += [(a, b) for a in (10, 11) for b in (12, 13)]
    g2 = scheme(5, P, N, edges); verify(5, list(P) + list(N), g2)
    return g2

SEG_A = [[("x", 0, 1), ("g", 0, 2)], [("g", 2, 5)], [("x", 1, 2), ("u", 0, 3)], [("u", 3, 5), ("g", 5, 10)],
         [("u", 5, 10)], [("g", 10, 13), ("u", 10, 13), ("t", 13, 14)], [("d", 0, 14)]]
SEG_B = [[("x", 0, 1), ("g", 0, 5)], [("x", 1, 2), ("u", 0, 3)], [("u", 3, 5), ("g", 5, 10)],
         [("u", 5, 10), ("g", 10, 13)], [("u", 10, 13), ("t", 13, 14)], [("d", 0, 14)]]
SEG_C = [[("x", 0, 1), ("g", 0, 3)], [("g", 3, 5), ("x", 1, 2), ("u", 0, 1)], [("u", 1, 5), ], [("g", 5, 10), ("u", 5, 10)],
         [("g", 10, 13), ("u", 10, 13), ("t", 13, 14)], [("d", 0, 14)]]

def make_v4(bm=512, o1="GU", o1f="GU", seg=SEG_A, osplit=(3,), scopes=False):
    R = bm // 2
    def fn(x, wg, wu, wd):
        B, S, D = x.shape
        F = wd.shape[0]
        nft = F // T
        tail = F - nft * T
        nb = S // bm
        xpat = {}; w1pat = {}
        def tables1(o):
            out = []
            for Pc, Nc, g, order in plan(o):
                ops = []
                for k in order:
                    u, v, w = g[k]
                    up, su = canon(u); vp, sv = canon(v)
                    xi = xpat.setdefault(up, len(xpat))
                    raw = len(vp) == 1 and vp[0][1] == 1
                    if not raw: w1pat.setdefault(vp, len(w1pat))
                    ops.append((up, vp, raw, {o: c * su * sv for o, c in w.items()}))
                out.append(ops)
            return out
        s1_first, s1_rest = tables1(o1f), tables1(o1)
        w2pat = {}; s2grp = {}
        for k, (u, v, w) in plan2().items():
            op, so_ = canon(u); hp, sh = canon(w); vp, sv = canon(v)
            raw = len(vp) == 1 and vp[0][1] == 1
            if not raw: w2pat.setdefault(vp, len(w2pat))
            s2grp.setdefault(op, []).append((hp, vp, raw, so_ * sh * sv))
        s2order = sorted(s2grp, key=lambda op: (min(i for (m, i), c in op), max(i for (m, i), c in op)))
        nseg = len(seg)
        segof = {}
        for si, sg in enumerate(seg):
            for kind, lo, hi in sg:
                for j in range(lo, hi): segof[(kind, j)] = si

        def kern(x_hbm, wg_hbm, wu_hbm, wd_hbm, o_hbm, xb, wgb, wub, wtb, wdb, wc1, wc2, xc, hb, ob, sem):
            def copies(si):
                out = []
                for kind, lo, hi in seg[si]:
                    if kind == "x":
                        out.append(pltpu.make_async_copy(x_hbm.at[pl.ds(lo*R, (hi-lo)*R)], xb.at[pl.ds(lo*R, (hi-lo)*R)], sem.at[si]))
                    elif kind in "gu":
                        src, dst = (wg_hbm, wgb) if kind == "g" else (wu_hbm, wub)
                        out.append(pltpu.make_async_copy(src.at[pl.ds(lo*T, (hi-lo)*T)], dst.at[pl.ds(lo*T, (hi-lo)*T)], sem.at[si]))
                    elif kind == "t":
                        out.append(pltpu.make_async_copy(wg_hbm.at[pl.ds(nft*T, tail)], wtb.at[pl.ds(0, tail)], sem.at[si]))
                        out.append(pltpu.make_async_copy(wu_hbm.at[pl.ds(nft*T, tail)], wtb.at[pl.ds(tail, tail)], sem.at[si]))
                    else:
                        n = min(hi*T, F) - lo*T
                        out.append(pltpu.make_async_copy(wd_hbm.at[pl.ds(lo*T, n)], wdb.at[pl.ds(lo*T, n)], sem.at[si]))
                return out
            cps = [copies(si) for si in range(nseg)]
            cx = pltpu.make_async_copy(x_hbm.at[pl.ds(bm, S - bm)], xb.at[pl.ds(bm, S - bm)], sem.at[nseg])
            for c in cps:
                for cp in c: cp.start()
            cx.start()
            wdb[pl.ds(F, T - tail), :] = jnp.zeros((T - tail, D), bf16)

            def w1raw(key):
                i, (kind, f) = key
                if kind == "t": return wtb[:, pl.ds(i*T, T)]
                return (wgb if kind == "g" else wub)[pl.ds(f*T, T), pl.ds(i*T, T)]
            def w2raw(key):
                i, f = key
                return wdb[pl.ds(f*T, T), pl.ds(i*T, T)]

            def block(i, first):
                r0 = 0 if first else pl.multiple_of(i * bm, bm)
                state = {"seg": 0}
                def need(items):
                    if not first: return
                    hi = max(segof[t] for t in items)
                    while state["seg"] <= hi:
                        for cp in cps[state["seg"]]: cp.wait()
                        state["seg"] += 1
                xraw = lambda k: xb[pl.ds(r0 + k[0]*R, R), pl.ds(k[1]*T, T)]
                xdone = {}
                def get_x(up):
                    if up in xdone: return xc[xpat[up]]
                    xdone[up] = True
                    if len(up) == 1 and up[0][1] == 1: v = xraw(up[0][0])
                    else: v = lincomb(up, lambda k: xraw(k).astype(f32)).astype(bf16)
                    xc[xpat[up]] = v
                    return v
                def get_w(vp, raw, rawf, pat, ref):
                    if raw: return rawf(vp[0][0])
                    if not first: return ref[pat[vp]]
                    v = lincomb(vp, lambda k: rawf(k).astype(f32)).astype(bf16)
                    ref[pat[vp]] = v
                    return v
                for ops in (s1_first if first else s1_rest):
                    acc = {}; left = {}; done = {}
                    for _, _, _, w in ops:
                        for o in w: left[o] = left.get(o, 0) + 1
                    for up, vp, raw, w in ops:
                        need([("x", k[0]) for k, c in up] + [k[1] for k, c in vp])
                        p = nt(get_x(up), get_w(vp, raw, w1raw, w1pat, wc1))
                        for o, c in w.items():
                            accum(acc, o, p, c)
                            left[o] -= 1
                            if left[o] == 0:
                                a, s = acc.pop(o)
                                assert s == 1
                                m, (kind, f) = o
                                if kind == "t": hb[m, f] = a * pltpu.roll(a, tail, 1)
                                elif (m, f) in done: hb[m, f] = done.pop((m, f)) * a
                                else: done[(m, f)] = a
                    assert not acc and not done
                acc = {}; left = {}
                for op in s2order:
                    for o, c in op: left[o] = left.get(o, 0) + 1
                bounds = [0] + list(osplit) + [D // T]
                nxt = 0
                for op in s2order:
                    p = None
                    for hp, vp, raw, s in sorted(s2grp[op], key=lambda t: -t[3]):
                        need([("d", k[1]) for k, c in vp])
                        lhs = lincomb(hp, lambda k: hb[k[0], k[1]]).astype(bf16)
                        q = nn(lhs, get_w(vp, raw, w2raw, w2pat, wc2))
                        if p is None: p, ps = q, s
                        elif s == ps: p = p + q
                        else: p = p - q
                    for o, c in op:
                        accum(acc, o, p, c * ps)
                        left[o] -= 1
                        if left[o] == 0:
                            a, s = acc.pop(o)
                            if s < 0: a = -a
                            ob[pl.ds(r0 + o[0]*R, R), pl.ds(o[1]*T, T)] = a.astype(bf16)
                    while nxt + 1 < len(bounds) and all(left[(m, j)] == 0 for m in (0, 1) for j in range(bounds[nxt], bounds[nxt+1])):
                        cs = pl.ds(bounds[nxt]*T, (bounds[nxt+1] - bounds[nxt])*T)
                        pltpu.make_async_copy(ob.at[pl.ds(r0, bm), cs], o_hbm.at[pl.ds(r0, bm), cs], sem.at[nseg + 1]).start()
                        nxt += 1

            block(0, True)
            cx.wait()
            lax.fori_loop(1, nb, lambda i, _: block(i, False), None)
            pltpu.make_async_copy(ob, o_hbm, sem.at[nseg + 1]).wait()

        out = pl.pallas_call(
            kern, in_specs=[ANY]*4, out_specs=ANY,
            out_shape=jax.ShapeDtypeStruct((S, D), x.dtype),
            scratch_shapes=[pltpu.VMEM((S, D), bf16), pltpu.VMEM((nft*T, D), bf16), pltpu.VMEM((nft*T, D), bf16),
                            pltpu.VMEM((T, D), bf16), pltpu.VMEM(((nft+1)*T, D), bf16),
                            pltpu.VMEM((len(w1pat), T, T), bf16), pltpu.VMEM((len(w2pat), T, T), bf16),
                            pltpu.VMEM((len(xpat), R, T), bf16), pltpu.VMEM((2, nft+1, R, T), f32),
                            pltpu.VMEM((S, D), bf16),
                            pltpu.SemaphoreType.DMA((nseg + 2,))],
            compiler_params=pltpu.CompilerParams(vmem_limit_bytes=100*1024*1024),
        )(x.reshape(S, D), wg.T, wu.T, wd)
        return out.reshape(B, S, D)
    return fn


@jax.jit
def pallas_standalone__glu_gated_bilinear__prompt_kernel(x, w_gate, w_up, w_down):
    return make_v4(osplit=(3, 4))(x, w_gate, w_up, w_down)
```

```python
import jax
import jax.numpy as jnp
import numpy as np
from jax import lax
import jax.experimental.pallas as pl
import jax.experimental.pallas.tpu as pltpu

TILE = 128
K_TILES = 5
F_TILES = 13
TAIL = 64
FIRST_BLOCK = 768
BLOCK = 640

F32 = jnp.float32
BF16 = jnp.bfloat16


_TEN = (
    [tuple(int(i == j) for j in range(K_TILES)) for i in range(K_TILES)] * 2,
    "PPPPPNNNNN",
    [(i, 5 + j, 1, -1) for i in range(5) for j in range(5) if i != j],
)
_SEVEN = (
    [(0, 0, 1, 0, 0), (1, 0, 0, -1, 0), (0, 0, 0, 1, 0), (0, 1, 0, 0, 0), (0, 0, 1, 0, -1),
     (1, 0, 0, 0, 0), (0, 0, 0, 0, 1)],
    "ZNPPZNP",
    [(0, 2, 1, 1), (0, 3, 1, 1), (1, 2, 1, 1), (1, 3, 1, 1), (8, 9, 1, 1), (7, 10, 1, 1),
     (4, 3, 1, 1), (4, 6, 1, 1), (5, 3, 1, 1), (5, 6, 1, 1), (13, 14, 1, 1), (12, 15, 1, 1),
     (6, 7, -1, 1), (15, 1, -1, -1), (4, 2, 1, 1)],
)

_PASSES = {
    "P": [((1, 0), (1, 1)), ((-1, 1), (0, 1))],
    "N": [((0, 1), (1, 1)), ((1, -1), (1, 0))],
    "Z": [((1, 0), (1, 0)), ((0, 1), (0, 1))],
}
_SEVENTH = {
    ("P", "N"): (((1, 0), (0, 1)), ((0, 1), (-1, 0))),
    ("Z", "P"): (((0, -1), (1, -1)), ((1, 0), (1, 1))),
    ("N", "Z"): (((-1, 1), (-1, 0)), ((-1, -1), (0, -1))),
}


def _products(scheme, columns):
    xs, colours, triples = scheme
    n = len(columns)
    points = [(np.array(xs[c]), np.eye(n, dtype=int)[c], colours[c]) for c in range(n)]
    passes = []
    for i, j, sx, sy in triples:
        first, second = points[i], (sx * points[j][0], sy * points[j][1], points[j][2])
        if (first[2], second[2]) not in _SEVENTH:
            first, second = second, first
        (u1, u2), (w1, w2) = _SEVENTH[first[2], second[2]]
        passes.append((np.outer(u1, first[0]) + np.outer(u2, second[0]),
                       np.outer(w1, first[1]) + np.outer(w2, second[1])))
        x, y = first[0] + second[0], first[1] + second[1]
        (colour,) = [c for c in "PNZ" if c not in (first[2], second[2])]
        if not any(c == colour and (abs(px + x).sum() == 0 or (px == x).all())
                   and (abs(py + y).sum() == 0 or (py == y).all()) for px, py, c in points):
            points.append((x, y, colour))
    for x, y, colour in points:
        passes += [(np.outer(u, x), np.outer(w, y)) for u, w in _PASSES[colour]]

    forms = np.array([np.outer(u, w).ravel() for u, w in passes]).T
    wanted = np.einsum("mp,ik,cd->mipckd", np.eye(2), np.eye(K_TILES), np.eye(n)).astype(int)
    wanted = wanted.reshape(len(forms), K_TILES * n)
    twice_v = np.rint(2 * np.linalg.lstsq(forms, wanted, rcond=None)[0]).astype(int)
    assert (forms @ twice_v == 2 * wanted).all(), "the passes do not add up to the matrix product"

    return [(
        {(m, i): int(u[m, i]) for m in (0, 1) for i in range(K_TILES) if u[m, i]},
        {(i, columns[c]): v[i, c] / 2 for i in range(K_TILES) for c in range(n) if v[i, c]},
        {(m, columns[c]): int(w[m, c]) for m in (0, 1) for c in range(n) if w[m, c]},
    ) for (u, w), v in zip(passes, twice_v.reshape(-1, K_TILES, n))]


def _normalised(coefficients):
    items = sorted(coefficients.items())
    sign = 1 if items[0][1] > 0 else -1
    return tuple((key, c * sign) for key, c in items), sign


def _with_both(coefficients, sign):
    out = {}
    for (m, tile), c in coefficients.items():
        if sign * coefficients.get((0, tile), 0) != coefficients.get((1, tile), 0):
            out[m, tile] = c
        elif m == 0:
            out[2, tile] = c
    return out


def _gate_up_passes():
    products = _products(_TEN, range(10)) + _products(_TEN, range(10, 20))
    products += _products(_SEVEN, range(20, 27))
    out, partial = [], {}
    for u, v, w in products:
        (u, su), (v, sv) = _normalised(u), _normalised(v)
        to = {key: c * su * sv for key, c in _with_both(w, 1).items()}
        partial.update({(m, c): {(0, c): 1, (1, c): 1} for m, c in to if m == 2})
        out.append((u, v, to))
    return out, partial


def _down_passes():
    scheme = ([x[::-1] for x in _SEVEN[0]],) + _SEVEN[1:]
    products = _products(scheme, range(7)) + _products(scheme, range(7, 14))
    out, partial = [], {}
    for u, v, w in products:
        (u, su), (v, sv), (w, sw) = _normalised(u), _normalised(v), _normalised(w)
        partial[u] = _with_both(dict(u), -1)
        partial.update({(m, i): {(0, i): 1, (1, i): -1} for m, i in partial[u] if m == 2})
        out.append((w, v, {u: su * sv * sw}))
    return out, partial


def _signed_sum(pattern, load):
    total = None
    for size in sorted({abs(c) for _, c in pattern}):
        terms = [(key, c) for key, c in pattern if abs(c) == size]
        sign = 1 if any(c > 0 for _, c in terms) else -1
        part = None
        for key, c in sorted(terms, key=lambda term: -sign * term[1]):
            value = load(key)
            part = value if part is None else part + value if sign * c > 0 else part - value
        if size != 1:
            part, sign = part * float(size * sign), 1
        if total is None:
            total = part if sign > 0 else -part
        else:
            total = total + part if sign > 0 else total - part
    return total


class _Accumulators:
    def __init__(self, passes, partial, finish):
        self.partial, self.finish, self.sums, self.missing = partial, finish, {}, {}
        for destinations in [to for _, _, to in passes] + list(partial.values()):
            for key in destinations:
                self.missing[key] = self.missing.get(key, 0) + 1

    def add(self, value, sign, destinations):
        for key, c in destinations.items():
            assert abs(c) == 1
            c *= sign
            if key not in self.sums:
                self.sums[key] = (value, c)
            else:
                total, s = self.sums[key]
                if s == c:
                    self.sums[key] = (total + value, s)
                else:
                    self.sums[key] = (total - value if s > 0 else value - total, 1)
            self.missing[key] -= 1
            if self.missing[key] == 0:
                total, s = self.sums.pop(key)
                if key in self.partial:
                    self.add(total, s, self.partial[key])
                else:
                    self.finish(key, total, s)


_GATE_UP_FIRST = [
    42, 20, 44, 46, 40, 22, 54, 50, 48, 58, 52, 60, 24, 56, 70, 62, 64, 76, 78, 68, 26, 4, 12, 31,
    8, 72, 30, 66, 28, 49, 74, 0, 17, 59, 32, 33, 41, 5, 35, 51, 34, 45, 61, 2, 36, 65, 77, 73, 79,
    25, 21, 14, 10, 1, 18, 69, 47, 138, 27, 63, 37, 55, 39, 7, 38, 9, 13, 71, 15, 148, 29, 19, 145,
    75, 134, 6, 89, 139, 112, 16, 120, 119, 95, 129, 98, 84, 143, 137, 102, 103, 87, 117, 85, 105,
    90, 128, 132, 140, 135, 141, 86, 130, 108, 158, 99, 164, 208, 113, 111, 211, 152, 154, 110,
    162, 177, 184, 123, 173, 178, 206, 121, 106, 100, 122, 212, 146, 107, 93, 81, 204, 115, 114,
    94, 170, 187, 118, 201, 149, 83, 127, 101, 210, 188, 194, 180, 11, 43, 3, 53, 57, 67, 125, 23,
    214, 186, 82, 133, 136, 104, 147, 88, 91, 157, 131, 155, 116, 163, 168, 182, 161, 175, 172,
    190, 166, 199, 80, 181, 183, 109, 153, 97, 176, 191, 189, 160, 167, 174, 179, 213, 151, 209,
    159, 96, 126, 200, 124, 92, 144, 150, 193, 203, 185, 207, 205, 169, 195, 171, 202, 192, 165,
    198, 196, 197, 142, 156,
]
_DOWN_FIRST = [
    32, 28, 104, 91, 13, 36, 103, 26, 83, 18, 74, 73, 81, 2, 100, 45, 41, 16, 46, 48, 42, 6, 21,
    72, 38, 5, 19, 50, 54, 70, 61, 59, 106, 15, 53, 60, 107, 109, 85, 52, 34, 39, 25, 78, 80, 31,
    23, 77, 56, 10, 65, 71, 12, 96, 79, 1, 8, 94, 24, 86, 66, 51, 43, 98, 40, 75, 95, 97, 69, 20,
    102, 55, 14, 62, 87, 105, 92, 82, 84, 37, 89, 29, 108, 101, 3, 58, 17, 7, 93, 27, 4, 11, 99,
    90, 9, 44, 63, 22, 35, 57, 76, 47, 64, 67, 30, 0, 68, 49, 33, 88,
]
_GATE_UP_ORDER = [
    32, 108, 193, 20, 28, 112, 64, 34, 114, 82, 124, 101, 100, 177, 211, 150, 104, 110, 136, 88,
    111, 21, 15, 39, 27, 106, 107, 35, 148, 94, 63, 210, 16, 184, 165, 117, 185, 116, 30, 166, 60,
    68, 99, 109, 73, 123, 151, 149, 179, 174, 205, 159, 127, 24, 11, 46, 62, 76, 18, 17, 192, 29,
    51, 77, 74, 145, 89, 93, 102, 115, 153, 98, 156, 137, 132, 86, 134, 49, 5, 14, 65, 182, 122,
    126, 130, 170, 167, 178, 8, 10, 25, 187, 213, 103, 183, 214, 52, 54, 72, 138, 160, 161, 66, 50,
    199, 1, 9, 176, 33, 196, 155, 198, 194, 113, 97, 3, 212, 181, 36, 58, 171, 186, 37, 188, 19,
    200, 38, 180, 162, 90, 203, 79, 168, 163, 140, 105, 143, 209, 175, 206, 71, 172, 195, 23, 70,
    6, 139, 26, 78, 7, 208, 173, 204, 53, 31, 55, 4, 2, 190, 47, 41, 141, 95, 75, 125, 121, 92,
    119, 59, 142, 0, 44, 40, 83, 118, 69, 85, 22, 56, 13, 154, 157, 96, 81, 84, 158, 146, 144, 67,
    42, 48, 135, 12, 45, 43, 57, 61, 131, 128, 91, 87, 120, 80, 147, 152, 207, 202, 169, 201, 129,
    191, 133, 164, 197, 189,
]
_DOWN_ORDER = [
    6, 83, 95, 64, 100, 45, 105, 82, 28, 50, 27, 40, 108, 23, 53, 69, 14, 79, 51, 74, 7, 67, 106,
    78, 49, 12, 62, 11, 104, 9, 24, 61, 94, 91, 52, 101, 66, 54, 109, 107, 57, 68, 46, 2, 39, 73,
    36, 18, 85, 19, 60, 30, 13, 55, 5, 72, 90, 3, 0, 84, 35, 58, 97, 75, 29, 20, 92, 102, 71, 87,
    17, 59, 103, 93, 48, 41, 38, 4, 65, 10, 31, 96, 16, 47, 37, 1, 70, 32, 56, 42, 98, 15, 86, 99,
    77, 22, 44, 63, 8, 43, 76, 21, 26, 81, 33, 89, 88, 80, 34, 25,
]

_LOADS = [
    [("x0", 0, 1), ("w", 0, 1)],
    [("w", 1, 2)],
    [("w", 2, 3)],
    [("w", 3, 4)],
    [("w", 4, 5)],
    [("x1", 0, 1), ("w", 5, 6)],
    [("x1", 1, 2), ("w", 6, 7)],
    [("x1", 2, 3), ("w", 7, 8)],
    [("x1", 3, 4), ("w", 8, 9)],
    [("x1", 4, 5), ("w", 9, 10)],
    [("w", 10, 13)],
    [("w", 13, 15), ("w", 15, 17)],
    [("w", 17, 20)],
    [("w", 20, 27)],
    [("d", 0, 1)],
    [("x", 0, 1)],
]
_STORE_TILES = [(0, 2), (2, 3), (3, 4)]
_LAST_TILE_CHUNKS = 4


def _is_one_tile(pattern):
    return len(pattern) == 1 and pattern[0][1] == 1


def _weight_sum_slots(passes):
    slots = {}
    for _, pattern, _ in passes:
        if not _is_one_tile(pattern):
            slots.setdefault(pattern, len(slots))
    return slots


def _tiles(lo, hi=None):
    return pl.ds(lo * TILE, ((lo + 1 if hi is None else hi) - lo) * TILE)


def _make_kernel(rows):
    gate_up, gate_up_partial = _gate_up_passes()
    down, down_partial = _down_passes()
    for order, passes in ((_GATE_UP_FIRST, gate_up), (_GATE_UP_ORDER, gate_up),
                          (_DOWN_FIRST, down), (_DOWN_ORDER, down)):
        assert sorted(order) == list(range(len(passes)))
    gate_up_slots, down_slots = _weight_sum_slots(gate_up), _weight_sum_slots(down)
    load_of = {
        (kind, j): n for n, load in enumerate(_LOADS) for kind, lo, hi in load for j in range(lo, hi)
    }
    f_full = F_TILES * TILE

    def body(x_hbm, wg_hbm, wu_hbm, wd_hbm, out_hbm,
             x_ref, w_ref, wd_ref, gate_up_sums, down_sums, out_ref, h_ref, sems):

        def copies(n):
            pairs = []
            for kind, lo, hi in _LOADS[n]:
                if kind == "x0":
                    part = (pl.ds(0, FIRST_BLOCK // 2),)
                    pairs.append((x_hbm.at[part], x_ref.at[part]))
                elif kind == "x1":
                    part = (pl.ds(FIRST_BLOCK // 2, FIRST_BLOCK // 2), _tiles(lo, hi))
                    pairs.append((x_hbm.at[part], x_ref.at[part]))
                elif kind == "x":
                    part = (pl.ds(FIRST_BLOCK, rows - FIRST_BLOCK),)
                    pairs.append((x_hbm.at[part], x_ref.at[part]))
                elif kind == "w" and hi <= 10:
                    pairs.append((wg_hbm.at[_tiles(lo, hi)], w_ref.at[_tiles(lo, hi)]))
                elif kind == "w" and hi <= 20:
                    pairs.append((wu_hbm.at[_tiles(lo - 10, hi - 10)], w_ref.at[_tiles(lo, hi)]))
                elif kind == "w":
                    for src, offset in ((wg_hbm, 0), (wu_hbm, TAIL)):
                        for c in range(lo, hi):
                            pairs.append((src.at[pl.ds(10 * TILE + (c - 20) * TAIL, TAIL)],
                                          w_ref.at[pl.ds(c * TILE + offset, TAIL)]))
                else:
                    pairs.append((wd_hbm, wd_ref.at[pl.ds(0, f_full + TAIL)]))
            return [pltpu.make_async_copy(src, dst, sems.at[n]) for src, dst in pairs]

        loads = [copies(n) for n in range(len(_LOADS))]
        for load in loads:
            for copy in load:
                copy.start()
        wd_ref[pl.ds(f_full + TAIL, TILE - TAIL), :] = jnp.zeros((TILE - TAIL, K_TILES * TILE), BF16)
        arrived = []

        def wait_for(items):
            while len(arrived) <= max(load_of[item] for item in items):
                for copy in loads[len(arrived)]:
                    copy.wait()
                arrived.append(True)

        def store(part):
            pltpu.make_async_copy(out_ref.at[part], out_hbm.at[part], sems.at[0]).start()

        def gate_up_tile(key):
            i, c = key
            return w_ref[_tiles(c), _tiles(i)]

        def down_tile(key):
            i, f = key
            return wd_ref[_tiles(f), _tiles(i)]

        def block(row0, first):
            half = (FIRST_BLOCK if first else BLOCK) // 2

            def weights(pattern, tile, slots, sums_ref):
                if _is_one_tile(pattern):
                    return tile(pattern[0][0])
                if not first:
                    return sums_ref[slots[pattern]].astype(BF16)
                value = _signed_sum(pattern, lambda key: tile(key).astype(F32))
                sums_ref[slots[pattern]] = value
                return value.astype(BF16)

            def x_tile(key):
                return x_ref[pl.ds(row0 + key[0] * half, half), _tiles(key[1])]

            x_sums, waiting, h_sign = {}, {}, {}

            def x_operand(pattern):
                if _is_one_tile(pattern):
                    return x_tile(pattern[0][0])
                if pattern not in x_sums:
                    total = _signed_sum(pattern, lambda key: x_tile(key).astype(F32))
                    x_sums[pattern] = total.astype(BF16)
                return x_sums[pattern]

            def finish_h(key, value, sign):
                m, c = key
                f = c % 10 if c < 20 else c // 2
                if f == F_TILES:
                    value, sign = value * pltpu.roll(value, TAIL, 1), 1
                elif (m, f) not in waiting:
                    waiting[m, f] = (value, sign)
                    return
                elif c < 20:
                    other, other_sign = waiting.pop((m, f))
                    value, sign = value * other, sign * other_sign
                else:
                    other, _ = waiting.pop((m, f))
                    a, b = (other, value) if c % 2 else (value, other)
                    low = lax.broadcasted_iota(jnp.int32, value.shape, 1) < TAIL
                    value, sign = jnp.where(low, a, b) * pltpu.roll(jnp.where(low, b, a), TAIL, 1), 1
                h_ref[f, pl.ds(m * half, half), :] = value
                h_sign[m, f] = sign

            sums = _Accumulators(gate_up, gate_up_partial, finish_h)
            for n in _GATE_UP_FIRST if first else _GATE_UP_ORDER:
                lhs, rhs, to = gate_up[n]
                if first:
                    wait_for([("x1", i) if m else ("x0", 0) for (m, i), _ in lhs]
                             + [("w", c) for (_, c), _ in rhs])
                product = lax.dot_general(
                    x_operand(lhs), weights(rhs, gate_up_tile, gate_up_slots, gate_up_sums),
                    (((1,), (1,)), ((), ())), preferred_element_type=F32)
                sums.add(product, 1, to)
            assert not sums.sums and not waiting

            finished, last_tile, h_both = [], {}, {}

            def finish_out(key, value, sign):
                m, j = key
                value = (value if sign > 0 else -value).astype(BF16)
                if first or j < K_TILES - 1:
                    out_ref[pl.ds(row0 + m * half, half), _tiles(j)] = value
                    finished.append(key)
                    return
                last_tile[m] = value
                if len(last_tile) == 2:
                    chunk = half // _LAST_TILE_CHUNKS
                    for start in range(0, half, chunk):
                        for side in (0, 1):
                            part = (pl.ds(row0 + side * half + start, chunk), _tiles(j))
                            out_ref[part] = last_tile[side][start:start + chunk]
                            store(part)

            def h_tile(key):
                m, f = key
                if m < 2:
                    return h_ref[f, pl.ds(m * half, half), :]
                if f not in h_both:
                    h_both[f] = h_tile((0, f)) + h_tile((1, f))
                return h_both[f]

            unsent = [(0, K_TILES)] if first else list(_STORE_TILES)
            sums = _Accumulators(down, down_partial, finish_out)
            for n in _DOWN_FIRST if first else _DOWN_ORDER:
                lhs, rhs, to = down[n]
                if first:
                    wait_for([("d", 0)])
                lhs, sign = _normalised({key: c * h_sign[key] for key, c in lhs})
                lhs = _signed_sum(tuple(_with_both(dict(lhs), 1).items()), h_tile)
                product = lax.dot_general(
                    lhs.astype(BF16), weights(rhs, down_tile, down_slots, down_sums),
                    (((1,), (0,)), ((), ())), preferred_element_type=F32)
                sums.add(product, sign, to)
                for lo, hi in list(unsent):
                    if all((m, j) in finished for m in (0, 1) for j in range(lo, hi)):
                        store((pl.ds(row0, 2 * half), _tiles(lo, hi)))
                        unsent.remove((lo, hi))
            assert not sums.sums and not unsent

        block(0, True)
        wait_for([("x", 0)])
        lax.fori_loop(
            0, (rows - FIRST_BLOCK) // BLOCK,
            lambda i, _: block(pl.multiple_of(FIRST_BLOCK + i * BLOCK, TILE), False), None)
        pltpu.make_async_copy(out_ref, out_hbm, sems.at[0]).wait()

    def kernel(*refs):
        pl.run_scoped(lambda sems: body(*refs, sems), pltpu.SemaphoreType.DMA((len(_LOADS),)))

    return kernel, len(gate_up_slots), len(down_slots)


@jax.jit
def pallas_standalone__glu_gated_bilinear__prompt_kernel(
    x: jax.Array,
    w_gate: jax.Array,
    w_up: jax.Array,
    w_down: jax.Array,
):
    batch, seq, d = x.shape
    rows = batch * seq
    assert d == K_TILES * TILE and w_down.shape == (F_TILES * TILE + TAIL, d)
    assert rows > FIRST_BLOCK and (rows - FIRST_BLOCK) % BLOCK == 0
    kernel, gate_up_sums, down_sums = _make_kernel(rows)

    hbm = pl.BlockSpec(memory_space=pl.ANY)
    out = pl.pallas_call(
        kernel,
        in_specs=[hbm] * 4,
        out_specs=hbm,
        out_shape=jax.ShapeDtypeStruct((rows, d), x.dtype),
        scratch_shapes=[
            pltpu.VMEM((rows, d), BF16),
            pltpu.VMEM(((2 * F_TILES + 1) * TILE, d), BF16),
            pltpu.VMEM(((F_TILES + 1) * TILE, d), BF16),
            pltpu.VMEM((gate_up_sums, TILE, TILE), F32),
            pltpu.VMEM((down_sums, TILE, TILE), F32),
            pltpu.VMEM((rows, d), BF16),
            pltpu.VMEM((F_TILES + 1, max(FIRST_BLOCK, BLOCK), TILE), F32),
        ],
        compiler_params=pltpu.CompilerParams(
            vmem_limit_bytes=64 * 1024 * 1024,
            flags={"XLA_TPU_RESCHEDULE_DMA_DONES": True},
        ),
    )(x.reshape(rows, d), w_gate.T, w_up.T, w_down)
    return out.reshape(batch, seq, d)
```
